```python
import os as _os
_os.environ.setdefault("JAX_PLATFORMS", "cpu")
import jax
import jax.numpy as jnp

def _softmax(x, axis=-1):
    return jax.nn.softmax(x, axis=axis)
def _gelu(x):
    return jax.nn.gelu(x, approximate=True)
def _silu(x):
    return jax.nn.silu(x)
def _sigmoid(x):
    return jax.nn.sigmoid(x)
def _layernorm(x, axis=-1, eps=1e-5):
    m = jnp.mean(x, axis=axis, keepdims=True)
    v = jnp.var(x, axis=axis, keepdims=True)
    return (x - m) / jnp.sqrt(v + eps)
def _scatter_add(tgt, idx, src, axis=0):
    return tgt.at[idx].add(src)
def _segment_sum(src, seg, n):
    return jax.ops.segment_sum(src, seg, n)
class _Rng:
    def __init__(self, key):
        self._k = key
    def _next(self):
        self._k, sub = jax.random.split(self._k)
        return sub
    def normal(self, shape):
        return jax.random.normal(self._next(), shape, dtype=jnp.bfloat16)
    def randint(self, lo, hi, shape):
        return jax.random.randint(self._next(), shape, lo, hi, dtype=jnp.int32)
    def uniform(self, shape, lo=0.0, hi=1.0):
        return jax.random.uniform(self._next(), shape, jnp.bfloat16, lo, hi)
    def permutation(self, n):
        return jax.random.permutation(self._next(), n)


kernel_name = 'concat_heads__mha_block_cached__mha_block_cached__near_ridge'

def setup_inputs():
    _rng = _Rng(jax.random.key(int.from_bytes(__import__("os").urandom(4), "little")))
    _w = (lambda a: (lambda t: t.astype(jnp.bfloat16) if jnp.issubdtype(t.dtype, jnp.floating) else t)(jnp.asarray(a)))
    def _A_setup():
        B, Sq, D = 8, 160, 512
        H, Sk, Dh = 32, 512, 128
        return {
            "x": _w((lambda *s: _rng.normal(s) * 0.8)(B, Sq, D)),
            "k_cache": _w((lambda *s: _rng.normal(s) * 0.8)(B, H, Sk, Dh)),
            "v_cache": _w((lambda *s: _rng.normal(s) * 0.05)(B, H, Sk, Dh)),
            "wq": _w((lambda *s: _rng.normal(s) * 0.8)(D, H * Dh) * (D ** -0.5)),
            "wo": _w((lambda *s: _rng.normal(s) * 0.05)(H * Dh, D) * ((H * Dh) ** -0.5)),
        }
    _A_in = _A_setup()

    def _B_setup():
        B, Sq, D = 8, 160, 512
        H, Sk, Dh = 32, 512, 128
        return {
            "x": _w((lambda *s: _rng.normal(s) * 0.8)(B, Sq, D)),
            "k_cache": _w((lambda *s: _rng.normal(s) * 0.8)(B, H, Sk, Dh)),
            "v_cache": _w((lambda *s: _rng.normal(s) * 0.05)(B, H, Sk, Dh)),
            "wq": _w((lambda *s: _rng.normal(s) * 0.8)(D, H * Dh) * (D ** -0.5)),
            "wo": _w((lambda *s: _rng.normal(s) * 0.05)(H * Dh, D) * ((H * Dh) ** -0.5)),
        }
    _B_in = _B_setup()

    return {
        "A_x": _A_in["x"],
        "A_k_cache": _A_in["k_cache"],
        "A_v_cache": _A_in["v_cache"],
        "A_wq": _A_in["wq"],
        "A_wo": _A_in["wo"],
        "B_x": _B_in["x"],
        "B_k_cache": _B_in["k_cache"],
        "B_v_cache": _B_in["v_cache"],
        "B_wq": _B_in["wq"],
        "B_wo": _B_in["wo"],
    }

def reference(A_x, A_k_cache, A_v_cache, A_wq, A_wo, B_x, B_k_cache, B_v_cache, B_wq, B_wo):
    def _A_ref(x, k_cache, v_cache, wq, wo):
        B, Sq, D = x.shape
        H, Dh = 32, 128
        q = (lambda x, *d: x.transpose(*d))((x @ wq).reshape(B, Sq, H, Dh), 0, 2, 1, 3)
        scores = jnp.einsum("bhqd,bhkd->bhqk", q, k_cache) * (Dh ** -0.5)
        p = _softmax(scores, axis=-1)
        o = jnp.einsum("bhqk,bhkd->bhqd", p, v_cache)
        return (lambda x, *d: x.transpose(*d))(o, 0, 2, 1, 3).reshape(B, Sq, H * Dh) @ wo

    def _B_ref(x, k_cache, v_cache, wq, wo):
        B, Sq, D = x.shape
        H, Dh = 32, 128
        q = (lambda x, *d: x.transpose(*d))((x @ wq).reshape(B, Sq, H, Dh), 0, 2, 1, 3)
        scores = jnp.einsum("bhqd,bhkd->bhqk", q, k_cache) * (Dh ** -0.5)
        p = _softmax(scores, axis=-1)
        o = jnp.einsum("bhqk,bhkd->bhqd", p, v_cache)
        return (lambda x, *d: x.transpose(*d))(o, 0, 2, 1, 3).reshape(B, Sq, H * Dh) @ wo

    a = _A_ref(A_x, A_k_cache, A_v_cache, A_wq, A_wo)
    b = _B_ref(B_x, B_k_cache, B_v_cache, B_wq, B_wo)
    return jnp.concatenate([a, b], axis=-1)
```

```python
import functools

import jax
import jax.numpy as jnp
from jax import lax
import jax.experimental.pallas as pl
import jax.experimental.pallas.tpu as pltpu

_B, _SQ, _D = 8, 160, 512
_H, _SK, _DH = 32, 512, 128
_G = 8
_NHG = _H // _G
_SCALE = float(_DH) ** -0.5


def _mha_part(x_ref, k_ref, v_ref, wq_ref, wo_ref):
    q = jnp.dot(x_ref[0], wq_ref[...], preferred_element_type=jnp.float32)
    q = (q * _SCALE).astype(jnp.bfloat16)
    outs = []
    for g in range(_G):
        qg = q[:, g * _DH:(g + 1) * _DH]
        s = lax.dot_general(qg, k_ref[0, g], (((1,), (1,)), ((), ())),
                            preferred_element_type=jnp.float32)
        m = jnp.max(s, axis=-1, keepdims=True)
        p = jnp.exp(s - m)
        l = jnp.sum(p, axis=-1, keepdims=True)
        o = jnp.dot(p.astype(jnp.bfloat16), v_ref[0, g],
                    preferred_element_type=jnp.float32)
        outs.append((o / l).astype(jnp.bfloat16))
    o_all = jnp.concatenate(outs, axis=-1)
    return jnp.dot(o_all, wo_ref[...], preferred_element_type=jnp.float32)


def _kernel(ax, ak, av, awq, awo, bx, bk, bv, bwq, bwo, o_ref, acc_ref):
    hg = pl.program_id(0)
    b = pl.program_id(1)
    ya = _mha_part(ax, ak, av, awq, awo)
    yb = _mha_part(bx, bk, bv, bwq, bwo)

    @pl.when(hg == 0)
    def _():
        acc_ref[b, :, 0:_D] = ya
        acc_ref[b, :, _D:2 * _D] = yb

    @pl.when(hg > 0)
    def _():
        acc_ref[b, :, 0:_D] += ya
        acc_ref[b, :, _D:2 * _D] += yb

    @pl.when(hg == _NHG - 1)
    def _():
        o_ref[b] = acc_ref[b].astype(o_ref.dtype)


@jax.jit
def pallas_concat_heads__mha_block_cached__mha_block_cached__near_ridge_kernel(
    A_x, A_k_cache, A_v_cache, A_wq, A_wo, B_x, B_k_cache, B_v_cache, B_wq, B_wo,
):
    part_specs = [
        pl.BlockSpec((1, _SQ, _D), lambda hg, b: (b, 0, 0)),
        pl.BlockSpec((1, _G, _SK, _DH), lambda hg, b: (b, hg, 0, 0)),
        pl.BlockSpec((1, _G, _SK, _DH), lambda hg, b: (b, hg, 0, 0)),
        pl.BlockSpec((_D, _G * _DH), lambda hg, b: (0, hg)),
        pl.BlockSpec((_G * _DH, _D), lambda hg, b: (hg, 0)),
    ]
    return pl.pallas_call(
        _kernel,
        grid=(_NHG, _B),
        in_specs=part_specs + part_specs,
        out_specs=pl.BlockSpec((_B, _SQ, 2 * _D), lambda hg, b: (0, 0, 0)),
        out_shape=jax.ShapeDtypeStruct((_B, _SQ, 2 * _D), jnp.bfloat16),
        scratch_shapes=[pltpu.VMEM((_B, _SQ, 2 * _D), jnp.float32)],
        compiler_params=pltpu.CompilerParams(
            dimension_semantics=("arbitrary", "arbitrary"),
            vmem_limit_bytes=100 * 1024 * 1024,
        ),
    )(A_x, A_k_cache, A_v_cache, A_wq, A_wo, B_x, B_k_cache, B_v_cache, B_wq, B_wo)
```

```python
import jax
import jax.numpy as jnp
from jax import lax
import jax.experimental.pallas as pl
import jax.experimental.pallas.tpu as pltpu

_B, _SQ, _D = 8, 160, 512
_H, _SK, _DH = 32, 512, 128
_G = 8
_NHG = _H // _G
_GD = _G * _DH
_NSTEP = _NHG * _B
_NBUF = 2
_LQ, _LP, _LO, _ORDER = 1, 1, 1, 'oqsp'
_QB = 1
_SCALE = float(_DH) ** -0.5


def _kernel(ax, ak, av, awq, awo, bx, bk, bv, bwq, bwo, out_hbm,
            kvbuf, wqbuf, wobuf, xbuf, obuf, acc_ref,
            kv_sems, w_sems, x_sems, o_sems):
    t = pl.program_id(0)
    hg = t // _B
    b = t % _B
    hbm = ((ax, ak, av, awq, awo), (bx, bk, bv, bwq, bwo))

    def kv_copy(step, part, which):
        slot = step % _NBUF
        src = hbm[part][1 + which].at[step % _B, pl.ds((step // _B) * _G, _G)]
        j = part * 2 + which
        return pltpu.make_async_copy(src, kvbuf.at[slot, j],
                                     kv_sems.at[slot * 4 + j])

    def wq_copy(h, part):
        ws = h % 2
        return pltpu.make_async_copy(hbm[part][3].at[:, pl.ds(h * _GD, _GD)],
                                     wqbuf.at[ws, part],
                                     w_sems.at[ws * 4 + part])

    def wo_copy(h, part):
        ws = h % 2
        return pltpu.make_async_copy(hbm[part][4].at[pl.ds(h * _GD, _GD), :],
                                     wobuf.at[ws, part],
                                     w_sems.at[ws * 4 + 2 + part])

    def x_copy(bb, part):
        return pltpu.make_async_copy(hbm[part][0].at[bb], xbuf.at[part, bb],
                                     x_sems.at[part])

    def out_copy(bb):
        return pltpu.make_async_copy(obuf.at[bb], out_hbm.at[bb], o_sems.at[bb])

    @pl.when(t == 0)
    def _():
        for part in range(2):
            x_copy(0, part).start()
            wq_copy(0, part).start()
        for part in range(2):
            kv_copy(0, part, 0).start()
            kv_copy(0, part, 1).start()
            wo_copy(0, part).start()

    @pl.when(hg == 0)
    def _():
        for part in range(2):
            x_copy(b, part).wait()

    @pl.when(b == 0)
    def _():
        for part in range(2):
            wq_copy(hg, part).wait()
            wo_copy(hg, part).wait()

    for part in range(2):
        kv_copy(t, part, 0).wait()
        kv_copy(t, part, 1).wait()

    @pl.when(t + 1 < _NSTEP)
    def _():
        for part in range(2):
            kv_copy(t + 1, part, 0).start()
            kv_copy(t + 1, part, 1).start()

    @pl.when(t + 1 < _B)
    def _():
        for part in range(2):
            x_copy(t + 1, part).start()

    for j in range(4):
        @pl.when(jnp.logical_and(b == 1 + j, hg + 1 < _NHG))
        def _():
            (wq_copy if j < 2 else wo_copy)(hg + 1, j % 2).start()

    slot = t % _NBUF
    ws = hg % 2

    def qproj(part):
        q = jnp.dot(xbuf[part, b], wqbuf[ws, part],
                    preferred_element_type=jnp.float32)
        return (q * _SCALE).astype(jnp.bfloat16)

    def qk(q, part, g):
        return lax.dot_general(q[:, g * _DH:(g + 1) * _DH],
                               kvbuf[slot, part * 2, g],
                               (((1,), (1,)), ((), ())),
                               preferred_element_type=jnp.float32)

    def softmax(s):
        m = jnp.max(s, axis=-1, keepdims=True)
        p = jnp.exp(s - m)
        l = jnp.sum(p, axis=-1, keepdims=True)
        return p.astype(jnp.bfloat16), l

    def pv(pl_, part, g):
        p, l = pl_
        o = jnp.dot(p, kvbuf[slot, part * 2 + 1, g],
                    preferred_element_type=jnp.float32)
        return (o / l).astype(jnp.bfloat16)

    def oproj(o, part, g, y):
        tt = jnp.dot(o, wobuf[ws, part, g * _DH:(g + 1) * _DH, :],
                     preferred_element_type=jnp.float32)
        lo = part * _D
        if g == 0:
            y = jnp.where(hg == 0, 0.0, acc_ref[b, :, lo:lo + _D])
        y = y + tt
        if g == _G - 1:
            acc_ref[b, :, lo:lo + _D] = y
            obuf[b, :, lo:lo + _D] = y.astype(obuf.dtype)
        return y

    items = [(part, g) for part in range(2) for g in range(_G)]
    n = len(items)
    qs = [qproj(0), None]
    S, P, O = {}, {}, {}
    y = None
    for i in range(-_LQ, n + _LO + _LP + 1):
        for stage in _ORDER:
            if stage == 'q':
                j = i + _LQ
                if j == _QB:
                    qs[1] = qproj(1)
                if 0 <= j < n:
                    S[j] = qk(qs[items[j][0]], *items[j])
            elif stage == 's':
                j = i
                if 0 <= j < n:
                    P[j] = softmax(S.pop(j))
            elif stage == 'p':
                j = i - _LP
                if 0 <= j < n:
                    O[j] = pv(P.pop(j), *items[j])
            elif stage == 'o':
                j = i - _LP - _LO
                if 0 <= j < n:
                    y = oproj(O.pop(j), *items[j], y)

    @pl.when(hg == _NHG - 1)
    def _():
        out_copy(b).start()

    @pl.when(t == _NSTEP - 1)
    def _():
        for bb in range(_B):
            out_copy(bb).wait()


@jax.jit
def pallas_concat_heads__mha_block_cached__mha_block_cached__near_ridge_kernel(
    A_x, A_k_cache, A_v_cache, A_wq, A_wo, B_x, B_k_cache, B_v_cache, B_wq, B_wo,
):
    bf16 = jnp.bfloat16
    return pl.pallas_call(
        _kernel,
        grid=(_NSTEP,),
        in_specs=[pl.BlockSpec(memory_space=pl.ANY)] * 10,
        out_specs=pl.BlockSpec(memory_space=pl.ANY),
        out_shape=jax.ShapeDtypeStruct((_B, _SQ, 2 * _D), bf16),
        scratch_shapes=[
            pltpu.VMEM((_NBUF, 4, _G, _SK, _DH), bf16),
            pltpu.VMEM((2, 2, _D, _GD), bf16),
            pltpu.VMEM((2, 2, _GD, _D), bf16),
            pltpu.VMEM((2, _B, _SQ, _D), bf16),
            pltpu.VMEM((_B, _SQ, 2 * _D), bf16),
            pltpu.VMEM((_B, _SQ, 2 * _D), jnp.float32),
            pltpu.SemaphoreType.DMA((_NBUF * 4,)),
            pltpu.SemaphoreType.DMA((8,)),
            pltpu.SemaphoreType.DMA((2,)),
            pltpu.SemaphoreType.DMA((_B,)),
        ],
        compiler_params=pltpu.CompilerParams(
            dimension_semantics=("arbitrary",),
            vmem_limit_bytes=100 * 1024 * 1024, disable_bounds_checks=True,
        ),
    )(A_x, A_k_cache, A_v_cache, A_wq, A_wo, B_x, B_k_cache, B_v_cache, B_wq, B_wo)
```

```python
import jax
import jax.numpy as jnp
from jax import lax
import jax.experimental.pallas as pl
import jax.experimental.pallas.tpu as pltpu

_B, _SQ, _D = 8, 160, 512
_H, _SK, _DH = 32, 512, 128
_G = 4
_NB = 4
_NHG = _H // _G
_NBQ = _B // _NB
_GD = _G * _DH
_PSTEP = _NHG * _NBQ
_NSTEP = 2 * _PSTEP
_SCALE = float(_DH) ** -0.5
_LQ, _LP, _LO, _ORDER = 1, 1, 1, 'oqsp'


def _kernel(ax, ak, av, awq, awo, bx, bk, bv, bwq, bwo, out_hbm,
            kvbuf, wqbuf, wobuf, xbuf, obuf, acc_ref,
            kv_sems, w_sems, x_sems, o_sems):
    t = pl.program_id(0)
    hbm = ((ax, ak, av, awq, awo), (bx, bk, bv, bwq, bwo))

    def coords(step):
        part = step // _PSTEP
        r = step % _PSTEP
        return part, r // _NBQ, r % _NBQ

    part, hg, bq = coords(t)

    def kv_copy(step, p, which):
        _, h, q = coords(step)
        slot = step % 2
        src = hbm[p][1 + which].at[pl.ds(q * _NB, _NB), pl.ds(h * _G, _G)]
        return pltpu.make_async_copy(src, kvbuf.at[slot, which],
                                     kv_sems.at[slot * 2 + which])

    def w_copy(widx, p, which):
        h = widx % _NHG
        ws = widx % 2
        if which == 0:
            return pltpu.make_async_copy(hbm[p][3].at[:, pl.ds(h * _GD, _GD)],
                                         wqbuf.at[ws], w_sems.at[ws * 2])
        return pltpu.make_async_copy(hbm[p][4].at[pl.ds(h * _GD, _GD), :],
                                     wobuf.at[ws], w_sems.at[ws * 2 + 1])

    def x_copy(p, q):
        return pltpu.make_async_copy(hbm[p][0].at[pl.ds(q * _NB, _NB)],
                                     xbuf.at[p, pl.ds(q * _NB, _NB)],
                                     x_sems.at[p * _NBQ + q])

    def out_copy(p, q):
        return pltpu.make_async_copy(
            obuf.at[p, pl.ds(q * _NB, _NB)],
            out_hbm.at[pl.ds(q * _NB, _NB), :, pl.ds(p * _D, _D)],
            o_sems.at[p * _NBQ + q])

    def per_part(pp, fn):
        for p in range(2):
            @pl.when(pp == p)
            def _():
                fn(p)

    widx = t // _NBQ

    @pl.when(t == 0)
    def _():
        x_copy(0, 0).start()
        w_copy(0, 0, 0).start()
        kv_copy(0, 0, 0).start()
        kv_copy(0, 0, 1).start()
        w_copy(0, 0, 1).start()

    for q in range(_NBQ):
        for p in range(2):
            @pl.when(t == p * _PSTEP + q)
            def _():
                x_copy(p, q).wait()

    def wait_step(p):
        @pl.when(bq == 0)
        def _():
            w_copy(widx, p, 0).wait()
            w_copy(widx, p, 1).wait()

        kv_copy(t, p, 0).wait()
        kv_copy(t, p, 1).wait()

    per_part(part, wait_step)

    @pl.when(t + 1 < _NSTEP)
    def _():
        def go(p):
            kv_copy(t + 1, p, 0).start()
            kv_copy(t + 1, p, 1).start()
        per_part((t + 1) // _PSTEP, go)

    for q in range(_NBQ):
        for p in range(2):
            if p * _PSTEP + q > 0:
                @pl.when(t + 1 == p * _PSTEP + q)
                def _():
                    x_copy(p, q).start()

    for which in range(2):
        @pl.when(jnp.logical_and(bq == which, (widx + 1) * _NBQ < _NSTEP))
        def _():
            per_part(((widx + 1) * _NBQ) // _PSTEP,
                     lambda p: w_copy(widx + 1, p, which).start())

    slot = t % 2
    ws = widx % 2

    xs = xbuf[part, pl.ds(bq * _NB, _NB)].reshape(_NB * _SQ, _D)
    q_all = jnp.dot(xs, wqbuf[ws], preferred_element_type=jnp.float32)
    q_all = (q_all * _SCALE).astype(jnp.bfloat16)

    def qk(bi, g):
        return lax.dot_general(q_all[bi * _SQ:(bi + 1) * _SQ, g * _DH:(g + 1) * _DH],
                               kvbuf[slot, 0, bi, g],
                               (((1,), (1,)), ((), ())),
                               preferred_element_type=jnp.float32)

    def softmax(s):
        m = jnp.max(s, axis=-1, keepdims=True)
        p = jnp.exp(s - m)
        l = jnp.sum(p, axis=-1, keepdims=True)
        return p.astype(jnp.bfloat16), l

    def pv(pl_, bi, g):
        p, l = pl_
        o = jnp.dot(p, kvbuf[slot, 1, bi, g], preferred_element_type=jnp.float32)
        return (o / l).astype(jnp.bfloat16)

    def oproj(o, bi, g, y):
        tt = jnp.dot(o, wobuf[ws, g * _DH:(g + 1) * _DH, :],
                     preferred_element_type=jnp.float32)
        bb = bq * _NB + bi
        if g == 0:
            y = jnp.where(hg == 0, 0.0, acc_ref[bb])
        y = y + tt
        if g == _G - 1:
            acc_ref[bb] = y
            obuf[part, bb] = y.astype(obuf.dtype)
        return y

    items = [(bi, g) for bi in range(_NB) for g in range(_G)]
    n = len(items)
    S, P, O = {}, {}, {}
    y = None
    for i in range(-_LQ, n + _LO + _LP + 1):
        for stage in _ORDER:
            if stage == 'q':
                j = i + _LQ
                if 0 <= j < n:
                    S[j] = qk(*items[j])
            elif stage == 's':
                j = i
                if 0 <= j < n:
                    P[j] = softmax(S.pop(j))
            elif stage == 'p':
                j = i - _LP
                if 0 <= j < n:
                    O[j] = pv(P.pop(j), *items[j])
            elif stage == 'o':
                j = i - _LP - _LO
                if 0 <= j < n:
                    y = oproj(O.pop(j), *items[j], y)

    for p in range(2):
        for q in range(_NBQ):
            @pl.when(t == p * _PSTEP + (_NHG - 1) * _NBQ + q)
            def _():
                out_copy(p, q).start()

    @pl.when(t == _NSTEP - 1)
    def _():
        for p in range(2):
            for q in range(_NBQ):
                out_copy(p, q).wait()


@jax.jit
def pallas_concat_heads__mha_block_cached__mha_block_cached__near_ridge_kernel(
    A_x, A_k_cache, A_v_cache, A_wq, A_wo, B_x, B_k_cache, B_v_cache, B_wq, B_wo,
):
    bf16 = jnp.bfloat16
    return pl.pallas_call(
        _kernel,
        grid=(_NSTEP,),
        in_specs=[pl.BlockSpec(memory_space=pl.ANY)] * 10,
        out_specs=pl.BlockSpec(memory_space=pl.ANY),
        out_shape=jax.ShapeDtypeStruct((_B, _SQ, 2 * _D), bf16),
        scratch_shapes=[
            pltpu.VMEM((2, 2, _NB, _G, _SK, _DH), bf16),
            pltpu.VMEM((2, _D, _GD), bf16),
            pltpu.VMEM((2, _GD, _D), bf16),
            pltpu.VMEM((2, _B, _SQ, _D), bf16),
            pltpu.VMEM((2, _B, _SQ, _D), bf16),
            pltpu.VMEM((_B, _SQ, _D), jnp.float32),
            pltpu.SemaphoreType.DMA((4,)),
            pltpu.SemaphoreType.DMA((4,)),
            pltpu.SemaphoreType.DMA((2 * _NBQ,)),
            pltpu.SemaphoreType.DMA((2 * _NBQ,)),
        ],
        compiler_params=pltpu.CompilerParams(
            dimension_semantics=("arbitrary",),
            vmem_limit_bytes=100 * 1024 * 1024,
            disable_bounds_checks=True,
        ),
    )(A_x, A_k_cache, A_v_cache, A_wq, A_wo, B_x, B_k_cache, B_v_cache, B_wq, B_wo)
```
